```python
import jax
import jax.numpy as jnp

def _softmax(x, axis=-1):
    return jax.nn.softmax(x, axis=axis)
def _gelu(x):
    return jax.nn.gelu(x, approximate=True)
def _silu(x):
    return jax.nn.silu(x)
def _sigmoid(x):
    return jax.nn.sigmoid(x)
def _layernorm(x, axis=-1, eps=1e-5):
    m = jnp.mean(x, axis=axis, keepdims=True)
    v = jnp.var(x, axis=axis, keepdims=True)
    return (x - m) / jnp.sqrt(v + eps)
def _scatter_add(tgt, idx, src, axis=0):
    return tgt.at[idx].add(src)
def _segment_sum(src, seg, n):
    return jax.ops.segment_sum(src, seg, n)
class _Rng:
    def __init__(self, key):
        self._k = key
    def _next(self):
        self._k, sub = jax.random.split(self._k)
        return sub
    def normal(self, shape):
        return jax.random.normal(self._next(), shape, dtype=jnp.bfloat16)
    def randint(self, lo, hi, shape):
        return jax.random.randint(self._next(), shape, lo, hi, dtype=jnp.int32)
    def uniform(self, shape, lo=0.0, hi=1.0):
        return jax.random.uniform(self._next(), shape, jnp.bfloat16, lo, hi)
    def permutation(self, n):
        return jax.random.permutation(self._next(), n)


kernel_name = 'interleave_layers__sliding_block_cached__moe_arch_mod__decode'

def setup_inputs():
    _rng = _Rng(jax.random.key(int.from_bytes(__import__("os").urandom(4), "little")))
    _w = (lambda a: (lambda t: t.astype(jnp.bfloat16) if jnp.issubdtype(t.dtype, jnp.floating) else t)(jnp.asarray(a)))
    def _A_setup():
        B, Sq, D = 4, 1, 640
        Hq, Hkv, Sk, Dh = 32, 32, 4096, 192
        assert Hq % Hkv == 0, (Hq, Hkv)
        return {
            "x": _w((lambda *s: _rng.normal(s) * 0.05)(B, Sq, D)),
            "k_cache": _w((lambda *s: _rng.normal(s) * 0.05)(B, Hkv, Sk, Dh)),
            "v_cache": _w((lambda *s: _rng.normal(s) * 0.05)(B, Hkv, Sk, Dh)),
            "wq": _w((lambda *s: _rng.normal(s) * 0.05)(D, Hq * Dh) * (D ** -0.5)),
            "wo": _w((lambda *s: _rng.normal(s) * 0.05)(Hq * Dh, D) * ((Hq * Dh) ** -0.5)),
        }
    _A_in = _A_setup()

    def _B_setup():
        B, S, D, F, C = 4, 1, 640, 1536, 1
        return {
            "x": _w((lambda *s: _rng.normal(s) * 0.05)(B, S, D)),
            "w_r": _w((lambda *s: _rng.normal(s) * 0.05)(D)),
            "w_gate": _w((lambda *s: _rng.normal(s) * 0.05)(D, F)),
            "w_up": _w((lambda *s: _rng.normal(s) * 0.05)(D, F)),
            "w_down": _w((lambda *s: _rng.normal(s) * 0.05)(F, D)),
        }
    _B_in = _B_setup()

    return {
        "A_x": _A_in["x"],
        "A_k_cache": _A_in["k_cache"],
        "A_v_cache": _A_in["v_cache"],
        "A_wq": _A_in["wq"],
        "A_wo": _A_in["wo"],
        "B_x": _B_in["x"],
        "B_w_r": _B_in["w_r"],
        "B_w_gate": _B_in["w_gate"],
        "B_w_up": _B_in["w_up"],
        "B_w_down": _B_in["w_down"],
    }

def reference(A_x, A_k_cache, A_v_cache, A_wq, A_wo, B_x, B_w_r, B_w_gate, B_w_up, B_w_down):
    def _A_ref(x, k_cache, v_cache, wq, wo):
        B, Sq, D = x.shape
        Hq, Dh = 32, 192
        Hkv, Sk = k_cache.shape[1], k_cache.shape[2]
        W = min(4096, max(256, Sk // 4))
        rep = Hq // Hkv
        q = (lambda x, *d: x.transpose(*d))((x @ wq).reshape(B, Sq, Hq, Dh), 0, 2, 1, 3)
        k = jnp.repeat(k_cache[:, :, Sk - W:, :], rep, axis=1)
        v = jnp.repeat(v_cache[:, :, Sk - W:, :], rep, axis=1)
        scores = jnp.einsum("bhqd,bhkd->bhqk", q, k) * (Dh ** -0.5)
        p = _softmax(scores, axis=-1)
        o = jnp.einsum("bhqk,bhkd->bhqd", p, v)
        return (lambda x, *d: x.transpose(*d))(o, 0, 2, 1, 3).reshape(B, Sq, Hq * Dh) @ wo

    def _B_ref(x, w_r, w_gate, w_up, w_down):
        B, S, D = x.shape
        C = 1
        r = x @ w_r
        idx = jnp.argsort(-r, axis=-1)[:, :C]
        idx_e = jnp.repeat(idx.reshape(B, C, 1), D, axis=2)
        x_sel = jnp.take_along_axis(x, idx_e, axis=1)
        g = _silu(x_sel @ w_gate)
        u = x_sel @ w_up
        y = (g * u) @ w_down
        r_sel = _sigmoid(jnp.take_along_axis(r, idx, axis=1))
        y = y * r_sel.reshape(B, C, 1)
        b_off = (jnp.arange(B) * S).reshape(B, 1)
        flat_idx = (idx + b_off).reshape(B * C)
        zero = (x * 0.0).reshape(B * S, D)
        upd = _scatter_add(zero, flat_idx, y.reshape(B * C, D), axis=0)
        return x + upd.reshape(B, S, D)

    x = A_x
    x = x + _A_ref(_layernorm(x, axis=-1), A_k_cache, A_v_cache, A_wq, A_wo)
    x = x + _B_ref(_layernorm(x, axis=-1), B_w_r, B_w_gate, B_w_up, B_w_down)
    x = x + _A_ref(_layernorm(x, axis=-1), A_k_cache, A_v_cache, A_wq, A_wo)
    x = x + _B_ref(_layernorm(x, axis=-1), B_w_r, B_w_gate, B_w_up, B_w_down)
    return x
```

```python
import jax
import jax.numpy as jnp
from jax import lax
import jax.experimental.pallas as pl
import jax.experimental.pallas.tpu as pltpu

HQ = 32
DH = 192
G = 8
NG = HQ // G
GR = G * DH
EPS = 1e-5


def _layernorm(x):
    m = jnp.mean(x, axis=-1, keepdims=True)
    d = x - m
    v = jnp.mean(d * d, axis=-1, keepdims=True)
    return d / jnp.sqrt(v + EPS)


def _kernel(x_hbm, wr_hbm, k_hbm, v_hbm, wq_hbm, wo_hbm, wg_hbm, wu_hbm, wd_hbm, o_ref,
            xin, wr, kbuf, vbuf, wq, wo, wg, wu, wd, xs, sem_small, sem_w, sem_k, sem_v,
            *, B, S, W, D, F):
    def kv_copy(hbm, buf, sem, b, g):
        return pltpu.make_async_copy(
            hbm.at[pl.ds((b * NG + g) * GR, GR), pl.ds(S - W, W)],
            buf.at[b, pl.ds(g * GR, GR), :],
            sem.at[b, g])

    c_x = pltpu.make_async_copy(x_hbm, xin, sem_small.at[0])
    c_wr = pltpu.make_async_copy(wr_hbm, wr, sem_small.at[1])
    c_wq = pltpu.make_async_copy(wq_hbm, wq, sem_w.at[0])
    c_wo = pltpu.make_async_copy(wo_hbm, wo, sem_w.at[1])
    c_wg = pltpu.make_async_copy(wg_hbm, wg, sem_w.at[2])
    c_wu = pltpu.make_async_copy(wu_hbm, wu, sem_w.at[3])
    c_wd = pltpu.make_async_copy(wd_hbm, wd, sem_w.at[4])

    c_x.start()
    c_wr.start()
    c_wq.start()

    def issue(i, c):
        b = i // NG
        g = i % NG

        @pl.when(i == NG)
        def _():
            c_wo.start()
            c_wg.start()
            c_wu.start()
            c_wd.start()

        kv_copy(k_hbm, kbuf, sem_k, b, g).start()
        kv_copy(v_hbm, vbuf, sem_v, b, g).start()
        return c

    lax.fori_loop(0, B * NG, issue, 0)

    c_x.wait()
    c_wr.wait()
    xs[0:B, :] = xin[...].astype(jnp.float32)
    c_wq.wait()

    row = lax.broadcasted_iota(jnp.int32, (8, GR), 0)
    col = lax.broadcasted_iota(jnp.int32, (8, GR), 1)
    diag = (col >= row * DH) & (col < row * DH + DH)
    scale = DH ** -0.5

    def layer_pair(it, carry):
        b = it // 2
        first_pass = (it % 2) == 0
        x = jnp.broadcast_to(xs[pl.ds(b, 1), :], (8, D))

        xn = _layernorm(x).astype(jnp.bfloat16)

        def group(g, y):
            r0 = pl.multiple_of(g * GR, GR)
            q = jnp.dot(xn, wq[:, pl.ds(r0, GR)], preferred_element_type=jnp.float32)
            qbd = jnp.where(diag, q, 0.0).astype(jnp.bfloat16)

            @pl.when(first_pass)
            def _():
                kv_copy(k_hbm, kbuf, sem_k, b, g).wait()

            s = jnp.dot(qbd, kbuf[b, pl.ds(r0, GR), :],
                        preferred_element_type=jnp.float32) * scale
            m = jnp.max(s, axis=1, keepdims=True)
            e = jnp.exp(s - m)
            p = (e / jnp.sum(e, axis=1, keepdims=True)).astype(jnp.bfloat16)

            @pl.when(first_pass)
            def _():
                kv_copy(v_hbm, vbuf, sem_v, b, g).wait()

            o = lax.dot_general(p, vbuf[b, pl.ds(r0, GR), :], (((1,), (1,)), ((), ())),
                                preferred_element_type=jnp.float32)
            obd = jnp.where(diag, o, 0.0).astype(jnp.bfloat16)

            @pl.when(it == 0)
            def _():
                @pl.when(g == 0)
                def _():
                    c_wo.wait()

            return y + jnp.dot(obd, wo[pl.ds(r0, GR), :], preferred_element_type=jnp.float32)

        y = lax.fori_loop(0, NG, group, jnp.zeros((8, D), jnp.float32))
        x = x + jnp.sum(y, axis=0, keepdims=True)

        @pl.when(it == 0)
        def _():
            c_wg.wait()
            c_wu.wait()
            c_wd.wait()

        xn32 = _layernorm(x)
        xn = xn32.astype(jnp.bfloat16)
        r = jnp.sum(xn32 * wr[...].astype(jnp.float32)[None, :], axis=-1, keepdims=True)
        gate = jnp.dot(xn, wg[...], preferred_element_type=jnp.float32)
        up = jnp.dot(xn, wu[...], preferred_element_type=jnp.float32)
        h = (gate * jax.nn.sigmoid(gate) * up).astype(jnp.bfloat16)
        yb = jnp.dot(h, wd[...], preferred_element_type=jnp.float32)
        x = x + (xn32 + yb * jax.nn.sigmoid(r))
        xs[pl.ds(b, 1), :] = x[0:1, :]
        return carry

    lax.fori_loop(0, 2 * B, layer_pair, 0)
    o_ref[...] = xs[0:B, :].astype(o_ref.dtype)


@jax.jit
def pallas_interleave_layers__sliding_block_cached__moe_arch_mod__decode_kernel(
    A_x: jax.Array,
    A_k_cache: jax.Array,
    A_v_cache: jax.Array,
    A_wq: jax.Array,
    A_wo: jax.Array,
    B_x: jax.Array,
    B_w_r: jax.Array,
    B_w_gate: jax.Array,
    B_w_up: jax.Array,
    B_w_down: jax.Array,
):
    del B_x
    B, Sq, D = A_x.shape
    _, Hkv, S, Dh = A_k_cache.shape
    assert Sq == 1 and Hkv == HQ and Dh == DH
    W = min(4096, max(256, S // 4))
    F = B_w_gate.shape[1]
    kt = jnp.swapaxes(A_k_cache, 2, 3).reshape(B * HQ * DH, S)
    vt = jnp.swapaxes(A_v_cache, 2, 3).reshape(B * HQ * DH, S)
    x2 = A_x.reshape(B, D)
    bf = jnp.bfloat16
    out = pl.pallas_call(
        lambda *refs: _kernel(*refs, B=B, S=S, W=W, D=D, F=F),
        out_shape=jax.ShapeDtypeStruct((B, D), A_x.dtype),
        in_specs=[pl.BlockSpec(memory_space=pl.ANY)] * 9,
        out_specs=pl.BlockSpec(memory_space=pltpu.VMEM),
        scratch_shapes=[
            pltpu.VMEM((B, D), bf),
            pltpu.VMEM((D,), bf),
            pltpu.VMEM((B, HQ * DH, W), bf),
            pltpu.VMEM((B, HQ * DH, W), bf),
            pltpu.VMEM((D, HQ * DH), bf),
            pltpu.VMEM((HQ * DH, D), bf),
            pltpu.VMEM((D, F), bf),
            pltpu.VMEM((D, F), bf),
            pltpu.VMEM((F, D), bf),
            pltpu.VMEM((8, D), jnp.float32),
            pltpu.SemaphoreType.DMA((2,)),
            pltpu.SemaphoreType.DMA((5,)),
            pltpu.SemaphoreType.DMA((B, NG)),
            pltpu.SemaphoreType.DMA((B, NG)),
        ],
        compiler_params=pltpu.CompilerParams(vmem_limit_bytes=127 * 1024 * 1024),
    )(x2, B_w_r, kt, vt, A_wq, A_wo, B_w_gate, B_w_up, B_w_down)
    return out.reshape(B, Sq, D)
```

```python
import jax
import jax.numpy as jnp
from jax import lax
import jax.experimental.pallas as pl
import jax.experimental.pallas.tpu as pltpu

HQ = 32
DH = 192
G = 8
NG = HQ // G
GR = G * DH
NP = HQ // 2
PR = 2 * DH
KS = 2
VKS = 2
VS = 3
VCH = (8, 4, 2, 1, 1)
VOFF = tuple(sum(VCH[:i]) for i in range(len(VCH)))
EPS = 1e-5
f32 = jnp.float32
bf16 = jnp.bfloat16
i32 = jnp.int32


def _layernorm(x):
    m = jnp.mean(x, axis=-1, keepdims=True)
    d = x - m
    v = jnp.mean(d * d, axis=-1, keepdims=True)
    return d / jnp.sqrt(v + EPS)


def _iotas(n):
    return lax.broadcasted_iota(i32, (8, n), 0), lax.broadcasted_iota(i32, (8, n), 1)


def _kernel(x_hbm, wr_hbm, k_hbm, v_hbm, wq_hbm, wo_hbm, wg_hbm, wu_hbm, wd_hbm, o_ref,
            xin, wr, kbuf, vtbuf, vfin, pbuf, wq, wo, wg, wu, wd, xs,
            sem_w, sem_k, sem_v, *, B, S, W, D):
    SW = W // KS
    VW = W // VKS

    def k_copy(b, g, j):
        return pltpu.make_async_copy(
            k_hbm.at[pl.ds((b * NG + g) * GR, GR), pl.ds(S - W + j * SW, SW)],
            kbuf.at[b, j, pl.ds(g * GR, GR), :], sem_k.at[b, g])

    def v_copy(b, c, j):
        r0, n = VOFF[c] * PR, VCH[c] * PR
        return pltpu.make_async_copy(
            v_hbm.at[pl.ds(b * HQ * DH + r0, n), pl.ds(S - W + j * VW, VW)],
            vtbuf.at[b % VS, j, pl.ds(r0, n), :], sem_v.at[b, c])

    weights = [(x_hbm, xin), (wr_hbm, wr)]
    weights += [(wq_hbm.at[:, pl.ds(g * GR, GR)], wq.at[g]) for g in range(NG)]
    weights += [(wo_hbm, wo), (wg_hbm, wg), (wu_hbm, wu), (wd_hbm, wd)]
    weights = [pltpu.make_async_copy(s, d, sem_w.at[i]) for i, (s, d) in enumerate(weights)]

    def issue_kv(lo, hi):
        def issue_k(b, c_):
            for g in range(NG):
                for j in range(KS):
                    k_copy(b, g, j).start()
            return c_

        def issue_b(b, c_):
            lax.fori_loop(b, b + 1, issue_k, 0)
            for c in range(len(VCH)):
                for j in range(VKS):
                    v_copy(b, c, j).start()
            return c_

        lax.fori_loop(lo, hi, issue_b, 0)

    for c in weights:
        c.start()
    issue_kv(0, VS)
    for c in weights:
        c.wait()
    xs[0:B, :] = xin[...].astype(f32)

    scale = DH ** -0.5
    row_g, col_g = _iotas(GR)
    diag_g = (col_g >= row_g * DH) & (col_g < row_g * DH + DH)

    def probs(b, xn, g):
        r0 = g * GR if isinstance(g, int) else pl.multiple_of(g * GR, GR)
        q = jnp.dot(xn, wq[g], preferred_element_type=f32)
        qbd = jnp.where(diag_g, q, 0.0).astype(bf16)
        s = jnp.concatenate(
            [jnp.dot(qbd, kbuf[b, j, pl.ds(r0, GR), :], preferred_element_type=f32)
             for j in range(KS)], axis=1) * scale
        m = jnp.max(s, axis=1, keepdims=True)
        e = jnp.exp(s - m)
        return (e / jnp.sum(e, axis=1, keepdims=True)).astype(bf16)

    def ffn(x):
        xn32 = _layernorm(x)
        xn = xn32.astype(bf16)
        r = jnp.sum(xn32 * wr[...].astype(f32)[None, :], axis=-1, keepdims=True)
        gate = jnp.dot(xn, wg[...], preferred_element_type=f32)
        up = jnp.dot(xn, wu[...], preferred_element_type=f32)
        h = (gate * jax.nn.sigmoid(gate) * up).astype(bf16)
        yb = jnp.dot(h, wd[...], preferred_element_type=f32)
        return x + (xn32 + yb * jax.nn.sigmoid(r))

    def attn_first(b, x):
        xn = _layernorm(x).astype(bf16)
        slot = b % VS

        def grp(g, c_):
            for j in range(KS):
                k_copy(b, g, j).wait()
            pbuf[g] = probs(b, xn, g)
            return c_

        lax.fori_loop(0, NG, grp, 0)

        row, col = _iotas(PR)
        rowsel = row - (col >= DH).astype(i32)

        def pair(i, y):
            for c in range(len(VCH)):
                @pl.when(i == VOFF[c])
                def _():
                    for j in range(VKS):
                        v_copy(b, c, j).wait()
            r0 = pl.multiple_of(i * PR, 128)
            p = pbuf[i // (G // 2)]
            vt = [vtbuf[slot, j, pl.ds(r0, PR), :] for j in range(VKS)]
            for t in range(PR // 128):
                tt = jnp.concatenate([v[t * 128:(t + 1) * 128, :].T for v in vt], axis=0)
                vfin[i * (PR // 128) + t] = pltpu.bitcast(tt, i32)
            o = sum(lax.dot_general(p[:, j * VW:(j + 1) * VW], vt[j], (((1,), (1,)), ((), ())),
                                    preferred_element_type=f32) for j in range(VKS))
            obd = jnp.where(rowsel == (i % (G // 2)) * 2, o, 0.0).astype(bf16)
            return y + jnp.dot(obd, wo[pl.ds(r0, PR), :], preferred_element_type=f32)

        y = lax.fori_loop(0, NP, pair, jnp.zeros((8, D), f32))
        return x + jnp.sum(y, axis=0, keepdims=True)

    def attn_second(b, x):
        xn = _layernorm(x).astype(bf16)
        y = None
        for g in range(NG):
            p = probs(b, xn, g)
            o = jnp.concatenate(
                [jnp.dot(p, pltpu.bitcast(vfin[g * (GR // 128) + t], bf16), preferred_element_type=f32)
                 for t in range(GR // 128)], axis=1)
            obd = jnp.where(diag_g, o, 0.0).astype(bf16)
            yg = jnp.dot(obd, wo[g * GR:(g + 1) * GR, :], preferred_element_type=f32)
            y = yg if y is None else y + yg
        return x + jnp.sum(y, axis=0, keepdims=True)

    def per_batch(b, c):
        x = jnp.broadcast_to(xs[pl.ds(b, 1), :], (8, D))
        x = attn_first(b, x)

        @pl.when(b == 0)
        def _():
            issue_kv(VS, B)

        x = ffn(x)
        x = attn_second(b, x)
        x = ffn(x)
        xs[pl.ds(b, 1), :] = x[0:1, :]
        return c

    lax.fori_loop(0, B, per_batch, 0)
    o_ref[...] = xs[0:B, :].astype(o_ref.dtype)


@jax.jit
def pallas_interleave_layers__sliding_block_cached__moe_arch_mod__decode_kernel(
    A_x: jax.Array,
    A_k_cache: jax.Array,
    A_v_cache: jax.Array,
    A_wq: jax.Array,
    A_wo: jax.Array,
    B_x: jax.Array,
    B_w_r: jax.Array,
    B_w_gate: jax.Array,
    B_w_up: jax.Array,
    B_w_down: jax.Array,
):
    del B_x
    B, Sq, D = A_x.shape
    _, Hkv, S, Dh = A_k_cache.shape
    assert Sq == 1 and Hkv == HQ and Dh == DH and B > VS
    W = min(4096, max(256, S // 4))
    F = B_w_gate.shape[1]
    kt = jnp.swapaxes(A_k_cache, 2, 3).reshape(B * HQ * DH, S)
    vt = jnp.swapaxes(A_v_cache, 2, 3).reshape(B * HQ * DH, S)
    out = pl.pallas_call(
        lambda *refs: _kernel(*refs, B=B, S=S, W=W, D=D),
        out_shape=jax.ShapeDtypeStruct((B, D), A_x.dtype),
        in_specs=[pl.BlockSpec(memory_space=pl.ANY)] * 9,
        out_specs=pl.BlockSpec(memory_space=pltpu.VMEM),
        scratch_shapes=[
            pltpu.VMEM((B, D), bf16),
            pltpu.VMEM((D,), bf16),
            pltpu.VMEM((B, KS, HQ * DH, W // KS), bf16),
            pltpu.VMEM((VS, VKS, HQ * DH, W // VKS), bf16),
            pltpu.VMEM((HQ * DH // 128, W // 2, 128), i32),
            pltpu.VMEM((NG, 8, W), bf16),
            pltpu.VMEM((NG, D, GR), bf16),
            pltpu.VMEM((HQ * DH, D), bf16),
            pltpu.VMEM((D, F), bf16),
            pltpu.VMEM((D, F), bf16),
            pltpu.VMEM((F, D), bf16),
            pltpu.VMEM((8, D), f32),
            pltpu.SemaphoreType.DMA((6 + NG,)),
            pltpu.SemaphoreType.DMA((B, NG)),
            pltpu.SemaphoreType.DMA((B, len(VCH))),
        ],
        compiler_params=pltpu.CompilerParams(vmem_limit_bytes=127 * 1024 * 1024),
    )(A_x.reshape(B, D), B_w_r, kt, vt, A_wq, A_wo, B_w_gate, B_w_up, B_w_down)
    return out.reshape(B, Sq, D)
```

```python
import jax
import jax.numpy as jnp
from jax import lax
import jax.experimental.pallas as pl
import jax.experimental.pallas.tpu as pltpu

HQ = 32
DH = 192
G = 8
NG = HQ // G
GR = G * DH
GT = GR // 128
NP = HQ // 2
PR = 2 * DH
CS = 2
LS = 3
VCH = (8, 4, 2, 1, 1)
VOFF = tuple(sum(VCH[:i]) for i in range(len(VCH)))
O_VPU = (0, 0, GT, 0)
U_VPU = 3
Q_COLS = 2
LAG, EVERY = 6, 3
EPS = 1e-5
f32 = jnp.float32
bf16 = jnp.bfloat16
i32 = jnp.int32


def _center(x):
    d = x - jnp.mean(x, axis=-1, keepdims=True)
    v = jnp.mean(d * d, axis=-1, keepdims=True)
    return d, 1.0 / jnp.sqrt(v + EPS)


def _iotas(n):
    return lax.broadcasted_iota(i32, (8, n), 0), lax.broadcasted_iota(i32, (8, n), 1)


def _words(x):
    return pltpu.bitcast(x, i32)


def _bf(x):
    return pltpu.bitcast(x, bf16)


def _run(gen):
    for _ in gen:
        pass


def _zip(main, rate, side, lead=0):
    done = object()
    for _ in range(lead):
        next(main, done)
    credit = 0.0
    while True:
        credit += rate
        while credit >= 1.0:
            credit -= 1.0
            next(main, done)
        if next(side, done) is done:
            break
    _run(main)


def _chain(*gens):
    for g in gens:
        yield from g


def _kernel(x_hbm, wr_hbm, k_hbm, v_hbm, wq_hbm, wo_hbm, wg_hbm, wu_hbm, wd_hbm, o_ref,
            xin, wr, kland, vland, pbuf, wq, wo, wg, wu, wd, xs, xcol, ocol,
            sem_w, sem_k, sem_v, *, B, S, W, D, F):
    CW = W // CS
    NJ = W // 128
    NT = D // 128
    NF = F // 128

    def k_copy(b, j):
        return pltpu.make_async_copy(
            k_hbm.at[pl.ds(b * HQ * DH, HQ * DH), pl.ds(S - W + j * CW, CW)],
            kland.at[b % LS, j], sem_k.at[b])

    def v_copy(b, c, j, r0, n):
        return pltpu.make_async_copy(
            v_hbm.at[pl.ds(b * HQ * DH + r0 * PR, n * PR), pl.ds(S - W + j * CW, CW)],
            vland.at[b % LS, j, pl.ds(r0 * PR, n * PR), :], sem_v.at[b, c])

    def issue(b, part):
        if part == 0:
            for j in range(CS):
                k_copy(b, j).start()
        elif b == B - 1:
            for c in range(len(VCH)):
                for j in range(CS):
                    v_copy(b, c, j, VOFF[c], VCH[c]).start()
        else:
            for j in range(CS):
                v_copy(b, 0, j, 0, NP).start()

    def ordered(fns):
        def body(i, c_):
            for n_, fn in enumerate(fns):
                pl.when(i == n_)(fn)
            return c_
        lax.fori_loop(0, len(fns), body, 0)

    def startup(wq_l, wo_l, wg_l, wu_l, wd_l):
        cps = [(x_hbm, xin), (wr_hbm, wr), (wq_hbm, wq_l), (wo_hbm, wo_l),
               (wg_hbm, wg_l), (wu_hbm, wu_l), (wd_hbm, wd_l)]
        cps = [pltpu.make_async_copy(s, d, sem_w.at[i]) for i, (s, d) in enumerate(cps)]
        for c in cps:
            c.start()
        ordered([(lambda b=b, p=p: issue(b, p)) for b in range(LS) for p in range(2)])
        for c in cps:
            c.wait()
        xs[0:B, :] = xin[...].astype(f32)

        def cols(dst, src):
            def body(j, c_):
                dst[j] = _words(src[:, pl.ds(pl.multiple_of(j * 128, 128), 128)])
                return c_
            lax.fori_loop(0, dst.shape[0], body, 0)

        def rows(dst, src, rb=256):
            def body(i, c_):
                r = pl.multiple_of(i * rb, rb)
                for n in range(dst.shape[0]):
                    dst[n, pl.ds(pl.multiple_of(i * (rb // 2), rb // 2), rb // 2), :] = _words(
                        src[pl.ds(r, rb), n * 128:(n + 1) * 128])
                return c_
            lax.fori_loop(0, src.shape[0] // rb, body, 0)

        cols(wq, wq_l)
        cols(wg, wg_l)
        cols(wu, wu_l)
        rows(wo, wo_l)
        rows(wd, wd_l)

    pl.run_scoped(startup, pltpu.VMEM((D, HQ * DH), bf16), pltpu.VMEM((HQ * DH, D), bf16),
                  pltpu.VMEM((D, F), bf16), pltpu.VMEM((D, F), bf16), pltpu.VMEM((F, D), bf16))

    scale = DH ** -0.5
    row_g, col_g = _iotas(GR)
    diag_g = (col_g >= row_g * DH) & (col_g < row_g * DH + DH)

    def mm(lhs, ref, j0, nj, r0):
        n = lhs.shape[1]
        return jnp.concatenate(
            [jnp.dot(lhs, _bf(ref[j0 + j, pl.ds(r0 // 2, n // 2), :]), preferred_element_type=f32)
             for j in range(nj)], axis=1)

    def mm_steps(lhs_of, ref, j0, nj, r0, toks, out, key):
        lhs = lhs_of()
        parts = []
        for j in range(nj):
            acc = None
            for kt in range(lhs.shape[1] // 128):
                t = jnp.dot(lhs[:, kt * 128:(kt + 1) * 128],
                            _bf(ref[j0 + j, r0 // 2 + kt * 64:r0 // 2 + (kt + 1) * 64, :]),
                            preferred_element_type=f32)
                acc = t if acc is None else acc + t
                toks.append(t)
                yield
            parts.append(acc)
        out[key] = jnp.concatenate(parts, axis=1)

    def to_columns(col_ref, row):
        for t in range(row.shape[1] // 128):
            col_ref[t * 128:(t + 1) * 128, :] = jnp.broadcast_to(
                row[0:1, t * 128:(t + 1) * 128], (128, 128)).T

    def vpu_steps(col_ref, ref, slabs, r0, nrows, accs, toks):
        for s in range(nrows // 16):
            cv = col_ref[s * 16:(s + 1) * 16, :]
            if s % EVERY == 0 and len(toks) > 0:
                z = toks[max(0, len(toks) - 1 - LAG)] * 0.0
                cv = cv + jnp.concatenate([z, z], axis=0)
            for j, sl in enumerate(slabs):
                w = _bf(ref[sl, r0 // 2 + s * 8:r0 // 2 + (s + 1) * 8, :]).astype(f32)
                v = w[0:8] * cv[0:8]
                a = v if accs[j] is None else accs[j] + v
                accs[j] = a + w[8:16] * cv[8:16]
            yield

    def row_sum(a):
        return jnp.broadcast_to(jnp.sum(a, axis=0, keepdims=True), a.shape)

    def softmax(s):
        m = jnp.max(s, axis=1, keepdims=True)
        e = jnp.exp(s - m)
        return (e / jnp.sum(e, axis=1, keepdims=True)).astype(bf16)

    def blockdiag(a):
        return jnp.where(diag_g, a, 0.0).astype(bf16)

    def ffn(x):
        d, inv = _center(x)
        db = d.astype(bf16)
        to_columns(xcol, db.astype(f32))
        toks, out, uacc = [], {}, [None] * U_VPU
        mxu = _chain(mm_steps(lambda: db, wg, 0, NF, 0, toks, out, 'gate'),
                     mm_steps(lambda: db, wu, 0, NF - U_VPU, 0, toks, out, 'up'))
        _zip(mxu, 1.15 * (2 * NF - U_VPU) * NT / (D // 16),
             vpu_steps(xcol, wu, range(NF - U_VPU, NF), 0, D, uacc, toks))
        gate = out['gate'] * inv
        up = jnp.concatenate([out['up']] + [row_sum(a) for a in uacc], axis=1) * inv
        r = jnp.sum(d * wr[...].astype(f32)[None, :], axis=-1, keepdims=True) * inv
        h = (gate * jax.nn.sigmoid(gate) * up).astype(bf16)
        yb = mm(h, wd, 0, NT, 0)
        return x + (d * inv + yb * jax.nn.sigmoid(r))

    def main(kfin, vfin):
        def attn_first(b, x):
            d, inv = _center(x)
            db = d.astype(bf16)
            slot = b % LS
            for j in range(CS):
                k_copy(b, j).wait()

            def grp(g, c_):
                qbd = blockdiag(mm(db, wq, g * GT, GT, 0))
                r0 = pl.multiple_of(g * GR, GR)
                parts = []
                for j in range(NJ):
                    kk = kland[slot, j // (CW // 128), pl.ds(r0, GR),
                               pl.ds((j % (CW // 128)) * 128, 128)]
                    kfin[j, pl.ds(pl.multiple_of(g * (GR // 2), GR // 2), GR // 2), :] = _words(kk)
                    parts.append(jnp.dot(qbd, kk, preferred_element_type=f32))
                pbuf[g] = softmax(jnp.concatenate(parts, axis=1) * (inv * scale))
                return c_

            lax.fori_loop(0, NG, grp, 0)

            row, col = _iotas(PR)
            rowsel = row - (col >= DH).astype(i32)

            def pair(i, y):
                for c in range(len(VCH)):
                    @pl.when((b == B - 1) & (i == VOFF[c]))
                    def _():
                        for j in range(CS):
                            v_copy(b, c, j, VOFF[c], VCH[c]).wait()

                @pl.when((b < B - 1) & (i == 0))
                def _():
                    for j in range(CS):
                        v_copy(b, 0, j, 0, NP).wait()

                r0 = pl.multiple_of(i * PR, 128)
                p = pbuf[i // (G // 2)]
                vt = [vland[slot, j, pl.ds(r0, PR), :] for j in range(CS)]
                for t in range(PR // 128):
                    vfin[i * (PR // 128) + t] = _words(jnp.concatenate(
                        [v[t * 128:(t + 1) * 128, :].T for v in vt], axis=0))
                o = sum(lax.dot_general(p[:, j * CW:(j + 1) * CW], vt[j], (((1,), (1,)), ((), ())),
                                        preferred_element_type=f32) for j in range(CS))
                obd = jnp.where(rowsel == (i % (G // 2)) * 2, o, 0.0).astype(bf16)
                return y + mm(obd, wo, 0, NT, r0)

            y = lax.fori_loop(0, NP, pair, jnp.zeros((8, D), f32))
            return x + jnp.sum(y, axis=0, keepdims=True)

        def attn_second(x):
            d, inv = _center(x)
            db = d.astype(bf16)
            to_columns(xcol, db.astype(f32))
            toks, out, yacc = [], {}, [None] * NT

            def q_vpu(g):
                parts = []
                for c0 in range(g * GT, (g + 1) * GT, Q_COLS):
                    accs = [None] * Q_COLS
                    yield from vpu_steps(xcol, wq, range(c0, c0 + Q_COLS), 0, D, accs, toks)
                    parts += [row_sum(a) for a in accs]
                out['q', g] = jnp.concatenate(parts, axis=1)

            def o_vpu(g):
                o = jnp.where(diag_g, out['o', g], 0.0)[:, :O_VPU[g] * 128]
                to_columns(ocol, row_sum(o).astype(bf16).astype(f32))
                yield from vpu_steps(ocol, wo, range(NT), g * GR, O_VPU[g] * 128, yacc, toks)

            def mxu(g):
                yield from mm_steps(lambda: blockdiag(out['q', g]), kfin, 0, NJ, g * GR,
                                    toks, out, ('s', g))
                yield from mm_steps(lambda: softmax(out['s', g] * (inv * scale)), vfin, g * GT, GT, 0,
                                    toks, out, ('o', g))
                if O_VPU[g] < GT:
                    yield from mm_steps(lambda: blockdiag(out['o', g])[:, O_VPU[g] * 128:], wo, 0, NT,
                                        g * GR + O_VPU[g] * 128, toks, out, ('y', g))

            _run(mm_steps(lambda: db, wq, 0, GT, 0, toks, out, ('q', 0)))
            assert O_VPU[-1] == 0
            for g in range(NG):
                side, ns = [], 0
                if g + 1 < NG:
                    side.append(q_vpu(g + 1))
                    ns += (GT // Q_COLS) * (D // 16)
                if g >= 1 and O_VPU[g - 1]:
                    side.append(o_vpu(g - 1))
                    ns += O_VPU[g - 1] * 8
                nm = 2 * NJ * GT + NT * (GT - O_VPU[g])
                lead, tail = (0, 40) if g + 1 < NG else (60, 0)
                _zip(mxu(g), (nm - lead - tail) / ns, _chain(*side), lead)
            y = jnp.concatenate(yacc, axis=1)
            for g in range(NG):
                if ('y', g) in out:
                    y = y + out['y', g]
            return x + jnp.sum(y, axis=0, keepdims=True)

        def per_batch(b, c):
            x = jnp.broadcast_to(xs[pl.ds(b, 1), :], (8, D))
            x = attn_first(b, x)
            x = ffn(x)
            x = attn_second(x)
            x = ffn(x)
            xs[pl.ds(b, 1), :] = x[0:1, :]
            pl.when(b == 0)(lambda: ordered([lambda: issue(B - 1, 0), lambda: issue(B - 1, 1)]))
            return c

        lax.fori_loop(0, B, per_batch, 0)

    pl.run_scoped(main, pltpu.VMEM((NJ, HQ * DH // 2, 128), i32),
                  pltpu.VMEM((HQ * DH // 128, W // 2, 128), i32))
    o_ref[...] = xs[0:B, :].astype(o_ref.dtype)


@jax.jit
def pallas_interleave_layers__sliding_block_cached__moe_arch_mod__decode_kernel(
    A_x: jax.Array,
    A_k_cache: jax.Array,
    A_v_cache: jax.Array,
    A_wq: jax.Array,
    A_wo: jax.Array,
    B_x: jax.Array,
    B_w_r: jax.Array,
    B_w_gate: jax.Array,
    B_w_up: jax.Array,
    B_w_down: jax.Array,
):
    del B_x
    B, Sq, D = A_x.shape
    _, Hkv, S, Dh = A_k_cache.shape
    assert Sq == 1 and Hkv == HQ and Dh == DH and B == LS + 1
    W = min(4096, max(256, S // 4))
    F = B_w_gate.shape[1]
    kt = jnp.swapaxes(A_k_cache, 2, 3).reshape(B * HQ * DH, S)
    vt = jnp.swapaxes(A_v_cache, 2, 3).reshape(B * HQ * DH, S)
    out = pl.pallas_call(
        lambda *refs: _kernel(*refs, B=B, S=S, W=W, D=D, F=F),
        out_shape=jax.ShapeDtypeStruct((B, D), A_x.dtype),
        in_specs=[pl.BlockSpec(memory_space=pl.ANY)] * 9,
        out_specs=pl.BlockSpec(memory_space=pltpu.VMEM),
        scratch_shapes=[
            pltpu.VMEM((B, D), bf16),
            pltpu.VMEM((D,), bf16),
            pltpu.VMEM((LS, CS, HQ * DH, W // CS), bf16),
            pltpu.VMEM((LS, CS, HQ * DH, W // CS), bf16),
            pltpu.VMEM((NG, 8, W), bf16),
            pltpu.VMEM((HQ * DH // 128, D // 2, 128), i32),
            pltpu.VMEM((D // 128, HQ * DH // 2, 128), i32),
            pltpu.VMEM((F // 128, D // 2, 128), i32),
            pltpu.VMEM((F // 128, D // 2, 128), i32),
            pltpu.VMEM((D // 128, F // 2, 128), i32),
            pltpu.VMEM((8, D), f32),
            pltpu.VMEM((D, 128), f32),
            pltpu.VMEM((GR, 128), f32),
            pltpu.SemaphoreType.DMA((7,)),
            pltpu.SemaphoreType.DMA((B,)),
            pltpu.SemaphoreType.DMA((B, len(VCH))),
        ],
        compiler_params=pltpu.CompilerParams(vmem_limit_bytes=127 * 1024 * 1024),
    )(A_x.reshape(B, D), B_w_r, kt, vt, A_wq, A_wo, B_w_gate, B_w_up, B_w_down)
    return out.reshape(B, Sq, D)
```
